```python
import os as _os
_os.environ.setdefault("JAX_PLATFORMS", "cpu")
import jax
import jax.numpy as jnp

def _softmax(x, axis=-1):
    return jax.nn.softmax(x, axis=axis)
def _gelu(x):
    return jax.nn.gelu(x, approximate=True)
def _silu(x):
    return jax.nn.silu(x)
def _sigmoid(x):
    return jax.nn.sigmoid(x)
def _layernorm(x, axis=-1, eps=1e-5):
    m = jnp.mean(x, axis=axis, keepdims=True)
    v = jnp.var(x, axis=axis, keepdims=True)
    return (x - m) / jnp.sqrt(v + eps)
def _scatter_add(tgt, idx, src, axis=0):
    return tgt.at[idx].add(src)
def _segment_sum(src, seg, n):
    return jax.ops.segment_sum(src, seg, n)
class _Rng:
    def __init__(self, key):
        self._k = key
    def _next(self):
        self._k, sub = jax.random.split(self._k)
        return sub
    def normal(self, shape):
        return jax.random.normal(self._next(), shape, dtype=jnp.bfloat16)
    def randint(self, lo, hi, shape):
        return jax.random.randint(self._next(), shape, lo, hi, dtype=jnp.int32)
    def uniform(self, shape, lo=0.0, hi=1.0):
        return jax.random.uniform(self._next(), shape, jnp.bfloat16, lo, hi)
    def permutation(self, n):
        return jax.random.permutation(self._next(), n)


kernel_name = 'concat_heads__mha_block_cached__mha_block_cached__near_ridge'

def setup_inputs():
    _rng = _Rng(jax.random.key(int.from_bytes(__import__("os").urandom(4), "little")))
    _w = (lambda a: (lambda t: t.astype(jnp.bfloat16) if jnp.issubdtype(t.dtype, jnp.floating) else t)(jnp.asarray(a)))
    def _A_setup():
        B, Sq, D = 16, 192, 512
        H, Sk, Dh = 32, 512, 128
        return {
            "x": _w((lambda *s: _rng.normal(s) * 0.8)(B, Sq, D)),
            "k_cache": _w((lambda *s: _rng.normal(s) * 0.8)(B, H, Sk, Dh)),
            "v_cache": _w((lambda *s: _rng.normal(s) * 0.05)(B, H, Sk, Dh)),
            "wq": _w((lambda *s: _rng.normal(s) * 0.8)(D, H * Dh) * (D ** -0.5)),
            "wo": _w((lambda *s: _rng.normal(s) * 0.05)(H * Dh, D) * ((H * Dh) ** -0.5)),
        }
    _A_in = _A_setup()

    def _B_setup():
        B, Sq, D = 16, 192, 512
        H, Sk, Dh = 32, 512, 128
        return {
            "x": _w((lambda *s: _rng.normal(s) * 0.8)(B, Sq, D)),
            "k_cache": _w((lambda *s: _rng.normal(s) * 0.8)(B, H, Sk, Dh)),
            "v_cache": _w((lambda *s: _rng.normal(s) * 0.05)(B, H, Sk, Dh)),
            "wq": _w((lambda *s: _rng.normal(s) * 0.8)(D, H * Dh) * (D ** -0.5)),
            "wo": _w((lambda *s: _rng.normal(s) * 0.05)(H * Dh, D) * ((H * Dh) ** -0.5)),
        }
    _B_in = _B_setup()

    return {
        "A_x": _A_in["x"],
        "A_k_cache": _A_in["k_cache"],
        "A_v_cache": _A_in["v_cache"],
        "A_wq": _A_in["wq"],
        "A_wo": _A_in["wo"],
        "B_x": _B_in["x"],
        "B_k_cache": _B_in["k_cache"],
        "B_v_cache": _B_in["v_cache"],
        "B_wq": _B_in["wq"],
        "B_wo": _B_in["wo"],
    }

def reference(A_x, A_k_cache, A_v_cache, A_wq, A_wo, B_x, B_k_cache, B_v_cache, B_wq, B_wo):
    def _A_ref(x, k_cache, v_cache, wq, wo):
        B, Sq, D = x.shape
        H, Dh = 32, 128
        q = (lambda x, *d: x.transpose(*d))((x @ wq).reshape(B, Sq, H, Dh), 0, 2, 1, 3)
        scores = jnp.einsum("bhqd,bhkd->bhqk", q, k_cache) * (Dh ** -0.5)
        p = _softmax(scores, axis=-1)
        o = jnp.einsum("bhqk,bhkd->bhqd", p, v_cache)
        return (lambda x, *d: x.transpose(*d))(o, 0, 2, 1, 3).reshape(B, Sq, H * Dh) @ wo

    def _B_ref(x, k_cache, v_cache, wq, wo):
        B, Sq, D = x.shape
        H, Dh = 32, 128
        q = (lambda x, *d: x.transpose(*d))((x @ wq).reshape(B, Sq, H, Dh), 0, 2, 1, 3)
        scores = jnp.einsum("bhqd,bhkd->bhqk", q, k_cache) * (Dh ** -0.5)
        p = _softmax(scores, axis=-1)
        o = jnp.einsum("bhqk,bhkd->bhqd", p, v_cache)
        return (lambda x, *d: x.transpose(*d))(o, 0, 2, 1, 3).reshape(B, Sq, H * Dh) @ wo

    a = _A_ref(A_x, A_k_cache, A_v_cache, A_wq, A_wo)
    b = _B_ref(B_x, B_k_cache, B_v_cache, B_wq, B_wo)
    return jnp.concatenate([a, b], axis=-1)
```

```python
import functools
import jax
import jax.numpy as jnp
from jax import lax
import jax.experimental.pallas as pl
import jax.experimental.pallas.tpu as pltpu

H, DH = 32, 128
LOG2E = 1.4426950408889634
NN = (((1,), (0,)), ((), ()))
NT = (((1,), (1,)), ((), ()))
F32 = jnp.float32
BF16 = jnp.bfloat16
QSCALE = DH ** -0.5 * LOG2E

def make(HG=4, NB=4, dA=2, dB=1, dD=1, pre=True):
    NG = H // HG
    W = HG * DH
    def kernel(xa, ka, va, wqa, woa, xb, kb, vb, wqb, wob, o_ref,
               xbuf, kvbuf, wqbuf, wobuf, qbuf, acc, xsem, kvsem, wqsem, wosem):
        bb = pl.program_id(0)
        hg = pl.program_id(1)
        nbb = pl.num_programs(0)
        step = bb * NG + hg
        nsteps = NG * nbb
        slot = step % 2
        gp = bb % 2
        Sq = 192
        D = 512
        X = (xa, xb); K = (ka, kb); V = (va, vb); WQ = (wqa, wqb); WO = (woa, wob)
        units = [(br, i, j) for i in range(NB) for j in range(HG) for br in range(2)]
        N = len(units)

        def x_cp(g, br):
            return pltpu.make_async_copy(X[br].at[pl.ds(g * (NB * Sq), NB * Sq), :], xbuf.at[g % 2, br], xsem.at[br])
        def wq_cp(h, br):
            return pltpu.make_async_copy(WQ[br].at[:, pl.ds(h * W, W)], wqbuf.at[br, h], wqsem.at[br, h])
        def wo_cp(h, br, sl):
            return pltpu.make_async_copy(WO[br].at[pl.ds(h * W, W), :], wobuf.at[br, h], wosem.at[sl, br])
        def start_kv(st, sl):
            h0 = (st % NG) * HG
            b0 = (st // NG) * NB
            for br in range(2):
                pltpu.make_async_copy(K[br].at[pl.ds(b0, NB), pl.ds(h0, HG)], kvbuf.at[sl, 2 * br], kvsem.at[sl]).start()
                pltpu.make_async_copy(V[br].at[pl.ds(b0, NB), pl.ds(h0, HG)], kvbuf.at[sl, 2 * br + 1], kvsem.at[sl]).start()
        def wait_kv(sl):
            pltpu.make_async_copy(kvbuf.at[sl], kvbuf.at[sl], kvsem.at[sl]).wait()

        @pl.when(step == 0)
        def _():
            def issue(t, carry):
                for br in range(2):
                    @pl.when(t == br)
                    def _():
                        x_cp(0, br).start()
                        wq_cp(0, br).start()
                @pl.when(jnp.logical_and(t >= 2, t <= NG))
                def _():
                    for br in range(2):
                        wq_cp(t - 1, br).start()
                for st in range(2):
                    @pl.when(t == NG + 1 + st)
                    def _():
                        start_kv(st, st)
                        for br in range(2):
                            wo_cp(st, br, st).start()
                return carry
            lax.fori_loop(0, NG + 3, issue, 0)
            if pre:
                def pbody(c, carry):
                    h = c // 2
                    br = c % 2
                    @pl.when(c < 2)
                    def _():
                        pltpu.make_async_copy(xbuf.at[0, br], xbuf.at[0, br], xsem.at[br]).wait()
                    pltpu.make_async_copy(wqbuf.at[br, h], wqbuf.at[br, h], wqsem.at[br, h]).wait()
                    r = lax.dot_general(xbuf[0, br], wqbuf[br, h], NN, preferred_element_type=F32)
                    qbuf[h, br] = (r * QSCALE).astype(BF16)
                    return carry
                lax.fori_loop(0, 2 * NG, pbody, 0)
            else:
                for br in range(2):
                    x_cp(0, br).wait()
                    for h in range(NG):
                        wq_cp(h, br).wait()

        @pl.when(jnp.logical_and(hg == 0, bb > 0))
        def _():
            for br in range(2):
                x_cp(bb, br).wait()
        @pl.when(bb == 0)
        def _():
            for br in range(2):
                wo_cp(hg, br, slot).wait()
        wait_kv(slot)

        def body(use_q):
            q = {}; p = {}; l = {}; o = {}
            first = hg == 0
            cnt = {}
            def A(u):
                br, i, j = units[u]
                if use_q:
                    q[u] = qbuf[hg, br, i * Sq:(i + 1) * Sq, j * DH:(j + 1) * DH]
                else:
                    w = wqbuf[br, hg, :, j * DH:(j + 1) * DH]
                    r = lax.dot_general(xbuf[gp, br, i * Sq:(i + 1) * Sq, :], w, NN, preferred_element_type=F32)
                    q[u] = (r * QSCALE).astype(BF16)
            def Bm(u):
                br, i, j = units[u]
                s = lax.dot_general(q[u], kvbuf[slot, 2 * br, i, j], NT, preferred_element_type=F32)
                m = jnp.max(s, axis=-1, keepdims=True)
                e = jnp.exp2(s - m)
                l[u] = jnp.sum(e, axis=-1, keepdims=True)
                p[u] = e.astype(BF16)
            def C(u):
                br, i, j = units[u]
                r = lax.dot_general(p[u], kvbuf[slot, 2 * br + 1, i, j], NN, preferred_element_type=F32)
                inv = pl.reciprocal(l[u], approx=True)
                inv = inv * (2.0 - l[u] * inv)
                o[u] = (r * inv).astype(BF16)
            def Dm(u):
                br, i, j = units[u]
                r = lax.dot_general(o[u], wobuf[br, hg, j * DH:(j + 1) * DH, :], NN, preferred_element_type=F32)
                prev = acc[i, :, br * D:(br + 1) * D]
                c = cnt.get((br, i), 0)
                cnt[(br, i)] = c + 1
                if c == 0:
                    prev = jnp.where(first, 0.0, prev)
                new = prev + r
                acc[i, :, br * D:(br + 1) * D] = new
                if c == HG - 1:
                    o_ref[i, :, br * D:(br + 1) * D] = new.astype(o_ref.dtype)
            for t in range(-dA, N + dD):
                if 0 <= t + dA < N: A(t + dA)
                if 0 <= t + dB < N: Bm(t + dB)
                if 0 <= t < N: C(t)
                if 0 <= t - dD < N: Dm(t - dD)
            @pl.when(step + 2 < nsteps)
            def _():
                start_kv(step + 2, slot)
            if use_q or not pre:
                @pl.when(step + 2 < NG)
                def _():
                    for br in range(2):
                        wo_cp(hg + 2, br, slot).start()
            @pl.when(jnp.logical_and(hg == 0, bb + 1 < nbb))
            def _():
                for br in range(2):
                    x_cp(bb + 1, br).start()

        if pre:
            @pl.when(bb == 0)
            def _():
                body(True)
            @pl.when(bb > 0)
            def _():
                body(False)
        else:
            body(False)

    def f(A_x, A_k, A_v, A_wq, A_wo, B_x, B_k, B_v, B_wq, B_wo):
        B, Sq, D = A_x.shape
        Sk = A_k.shape[2]
        anyspec = pl.BlockSpec(memory_space=pl.ANY)
        return pl.pallas_call(
            kernel,
            grid=(B // NB, NG),
            in_specs=[anyspec] * 10,
            out_specs=pl.BlockSpec((NB, Sq, 2 * D), lambda b, g: (b, 0, 0)),
            out_shape=jax.ShapeDtypeStruct((B, Sq, 2 * D), jnp.bfloat16),
            scratch_shapes=[
                pltpu.VMEM((2, 2, NB * Sq, D), BF16),
                pltpu.VMEM((2, 4, NB, HG, Sk, DH), BF16),
                pltpu.VMEM((2, NG, D, W), BF16),
                pltpu.VMEM((2, NG, W, D), BF16),
                pltpu.VMEM((NG, 2, NB * Sq, W), BF16),
                pltpu.VMEM((NB, Sq, 2 * D), F32),
                pltpu.SemaphoreType.DMA((2,)),
                pltpu.SemaphoreType.DMA((2,)),
                pltpu.SemaphoreType.DMA((2, NG)),
                pltpu.SemaphoreType.DMA((2, 2)),
            ],
            compiler_params=pltpu.CompilerParams(
                dimension_semantics=("arbitrary", "arbitrary"),
                vmem_limit_bytes=110 * 1024 * 1024, disable_bounds_checks=True),
        )(A_x.reshape(B * Sq, D), A_k, A_v, A_wq, A_wo, B_x.reshape(B * Sq, D), B_k, B_v, B_wq, B_wo)
    return f

_impl = make()


@jax.jit
def pallas_concat_heads__mha_block_cached__mha_block_cached__near_ridge_kernel(
    A_x, A_k_cache, A_v_cache, A_wq, A_wo, B_x, B_k_cache, B_v_cache, B_wq, B_wo
):
    return _impl(A_x, A_k_cache, A_v_cache, A_wq, A_wo, B_x, B_k_cache, B_v_cache, B_wq, B_wo)
```

```python
import functools
import jax
import jax.numpy as jnp
from jax import lax
import jax.experimental.pallas as pl
import jax.experimental.pallas.tpu as pltpu

H, DH = 32, 128
LOG2E = 1.4426950408889634
NN = (((1,), (0,)), ((), ()))
NT = (((1,), (1,)), ((), ()))
F32 = jnp.float32
BF16 = jnp.bfloat16
QSCALE = DH ** -0.5 * LOG2E
SQ, DM, SK, NBATCH = 192, 512, 512, 16
ORDER = (("C", 0), ("B", 1), ("A", 2), ("D", -1))
ORDER_Q = (("A", 3), ("D", -1), ("B", 1), ("C", 0))

def make(HG=4, NB=4, KP=5, S2=10, order=ORDER, order_q=ORDER_Q, order2=None, only=None):
    NS = 4
    NG = H // HG
    W = HG * DH
    NBB = NBATCH // NB
    NSTEPS = NBB * NG
    LOG_NG = NG.bit_length() - 1
    assert KP >= NS and KP <= NG and S2 >= NG and S2 % 2 == 0 and S2 <= NSTEPS

    def kernel(xa, ka, va, wqa, woa, xb, kb, vb, wqb, wob, o_ref,
               xbuf, kvbuf, wqbuf, wobuf, qbuf, acc, obuf, x0sem, xsem, kvsem, wq0sem, wqsem, wosem, osem):
        X = (xa, xb); K = (ka, kb); V = (va, vb); WQ = (wqa, wqb); WO = (woa, wob)

        def wait(ref, sem):
            pltpu.make_async_copy(ref, ref, sem).wait()
        def x_cp(g, br, sem):
            return pltpu.make_async_copy(X[br].at[pl.ds(g * (NB * SQ), NB * SQ), :], xbuf.at[g & 1, br], sem)
        def wq_cp(h, br, sem):
            return pltpu.make_async_copy(WQ[br].at[:, pl.ds(h * W, W)], wqbuf.at[h, br], sem)
        def start_wo(h):
            for br in range(2):
                pltpu.make_async_copy(WO[br].at[pl.ds(h * W, W), :], wobuf.at[h, br], wosem.at[h & (NS - 1)]).start()
        def start_kv(st):
            sl = st & (NS - 1)
            h0 = (st & (NG - 1)) * HG
            b0 = (st >> LOG_NG) * NB
            for br in range(2):
                pltpu.make_async_copy(K[br].at[pl.ds(b0, NB), pl.ds(h0, HG)], kvbuf.at[sl, 2 * br], kvsem.at[sl]).start()
                pltpu.make_async_copy(V[br].at[pl.ds(b0, NB), pl.ds(h0, HG)], kvbuf.at[sl, 2 * br + 1], kvsem.at[sl]).start()

        def issue(t, carry):
            for br in range(2):
                @pl.when(t == br)
                def _():
                    x_cp(0, br, x0sem.at[br]).start()
                    wq_cp(0, br, wq0sem.at[0, br]).start()
            @pl.when(jnp.logical_and(t >= 2, t <= KP))
            def _():
                for br in range(2):
                    wq_cp(t - 1, br, wq0sem.at[t - 1, br]).start()
            @pl.when(t > KP)
            def _():
                st = t - (KP + 1)
                start_kv(st)
                start_wo(st)
            return carry
        lax.fori_loop(0, KP + 1 + NS, issue, 0)

        def pbody(c, carry):
            h = c >> 1
            br = c & 1
            @pl.when(c < 2)
            def _():
                wait(xbuf.at[0, br], x0sem.at[br])
            wait(wqbuf.at[h, br], wq0sem.at[h, br])
            r = lax.dot_general(xbuf[0, br], wqbuf[h, br], NN, preferred_element_type=F32)
            qbuf[h, br] = (r * QSCALE).astype(BF16)
            return carry
        if only is None: lax.fori_loop(0, 2 * KP, pbody, 0)

        def body(step, use_q, nh, early):
            units = [(br, i, hh, j) for i in range(NB) for hh in range(nh) for j in range(HG) for br in range(2)]
            N = len(units)
            bb = step >> LOG_NG
            hg = step & (NG - 1)
            gp = bb & 1
            slots = [(step + hh) & (NS - 1) for hh in range(nh)]
            if use_q:
                wait(wobuf.at[hg], wosem.at[slots[0]])
            else:
                if early:
                    @pl.when(step < NG)
                    def _():
                        wait(wobuf.at[hg], wosem.at[slots[0]])
                        wait(wqbuf.at[hg], wqsem.at[slots[0]])
                @pl.when(hg == 0)
                def _():
                    wait(xbuf.at[gp], xsem)
                @pl.when(jnp.logical_and(hg == 0, bb >= 2))
                def _():
                    wait(obuf.at[gp], osem.at[gp])
            for sl in slots:
                wait(kvbuf.at[sl], kvsem.at[sl])

            q = {}; p = {}; l = {}; o = {}
            first = hg == 0
            cnt = {}
            def A(u):
                br, i, hh, j = units[u]
                if use_q:
                    q[u] = qbuf[hg, br, i * SQ:(i + 1) * SQ, j * DH:(j + 1) * DH]
                else:
                    w = wqbuf[hg + hh, br, :, j * DH:(j + 1) * DH]
                    r = lax.dot_general(xbuf[gp, br, i * SQ:(i + 1) * SQ, :], w, NN, preferred_element_type=F32)
                    q[u] = (r * QSCALE).astype(BF16)
            def Bm(u):
                br, i, hh, j = units[u]
                s = lax.dot_general(q[u], kvbuf[slots[hh], 2 * br, i, j], NT, preferred_element_type=F32)
                m = jnp.max(s, axis=-1, keepdims=True)
                e = jnp.exp2(s - m)
                l[u] = jnp.sum(e, axis=-1, keepdims=True)
                p[u] = e.astype(BF16)
            def C(u):
                br, i, hh, j = units[u]
                r = lax.dot_general(p[u], kvbuf[slots[hh], 2 * br + 1, i, j], NN, preferred_element_type=F32)
                inv = pl.reciprocal(l[u], approx=True)
                inv = inv * (2.0 - l[u] * inv)
                o[u] = (r * inv).astype(BF16)
            def Dm(u):
                br, i, hh, j = units[u]
                r = lax.dot_general(o[u], wobuf[hg + hh, br, j * DH:(j + 1) * DH, :], NN, preferred_element_type=F32)
                prev = acc[i, :, br * DM:(br + 1) * DM]
                c = cnt.get((br, i), 0)
                cnt[(br, i)] = c + 1
                if c == 0:
                    prev = jnp.where(first, 0.0, prev)
                new = prev + r
                acc[i, :, br * DM:(br + 1) * DM] = new
                if c == nh * HG - 1 and (not use_q or KP == NG):
                    obuf[gp, i, :, br * DM:(br + 1) * DM] = new.astype(BF16)
                    if br == 1:
                        @pl.when(hg == NG - nh)
                        def _():
                            pltpu.make_async_copy(obuf.at[gp, i], o_ref.at[bb * NB + i], osem.at[gp]).start()
            fns = {"A": A, "B": Bm, "C": C, "D": Dm}
            od = order_q if use_q else (order2 if (nh == 2 and order2 is not None) else order)
            lo = -max(o_ for _, o_ in od)
            hi = N - min(o_ for _, o_ in od)
            for t in range(lo, hi):
                for st_, o_ in od:
                    if 0 <= t + o_ < N:
                        fns[st_](t + o_)
            for hh in range(nh):
                nxt = step + hh + NS
                @pl.when(nxt < NSTEPS)
                def _():
                    start_kv(nxt)
                if early:
                    @pl.when(nxt < NG)
                    def _():
                        start_wo(nxt)
                    @pl.when(jnp.logical_and(nxt >= KP, nxt < NG))
                    def _():
                        for br in range(2):
                            wq_cp(nxt, br, wqsem.at[nxt & (NS - 1)]).start()
                @pl.when(jnp.logical_and((nxt & (NG - 1)) == 0, nxt < NSTEPS))
                def _():
                    for br in range(2):
                        x_cp(nxt >> LOG_NG, br, xsem).start()

        def loop1(step, c):
            body(step, True, 1, True)
            return c
        if only in (None, 'bcd'): lax.fori_loop(0, KP, loop1, 0)
        def loop2(step, c):
            body(step, False, 1, True)
            return c
        if only in (None, 'full') and S2 > KP: lax.fori_loop(KP, S2, loop2, 0)
        def loop3(k, c):
            body(S2 + 2 * k, False, 2, False)
            return c
        if only in (None, 'full2') and S2 < NSTEPS: lax.fori_loop(0, (NSTEPS - S2) // 2, loop3, 0)
        wait(obuf.at[0], osem.at[0])
        wait(obuf.at[1], osem.at[1])

    def f(A_x, A_k, A_v, A_wq, A_wo, B_x, B_k, B_v, B_wq, B_wo):
        B, Sq, D = A_x.shape
        anyspec = pl.BlockSpec(memory_space=pl.ANY)
        return pl.pallas_call(
            kernel,
            in_specs=[anyspec] * 10,
            out_specs=anyspec,
            out_shape=jax.ShapeDtypeStruct((B, Sq, 2 * D), jnp.bfloat16),
            scratch_shapes=[
                pltpu.VMEM((2, 2, NB * SQ, DM), BF16),
                pltpu.VMEM((NS, 4, NB, HG, SK, DH), BF16),
                pltpu.VMEM((NG, 2, DM, W), BF16),
                pltpu.VMEM((NG, 2, W, DM), BF16),
                pltpu.VMEM((KP, 2, NB * SQ, W), BF16),
                pltpu.VMEM((NB, SQ, 2 * DM), F32),
                pltpu.VMEM((2, NB, SQ, 2 * DM), BF16),
                pltpu.SemaphoreType.DMA((2,)),
                pltpu.SemaphoreType.DMA(()),
                pltpu.SemaphoreType.DMA((NS,)),
                pltpu.SemaphoreType.DMA((KP, 2)),
                pltpu.SemaphoreType.DMA((NS,)),
                pltpu.SemaphoreType.DMA((NS,)),
                pltpu.SemaphoreType.DMA((2,)),
            ],
            compiler_params=pltpu.CompilerParams(
                vmem_limit_bytes=110 * 1024 * 1024, disable_bounds_checks=True,
                disable_semaphore_checks=True),
        )(A_x.reshape(B * Sq, D), A_k, A_v, A_wq, A_wo, B_x.reshape(B * Sq, D), B_k, B_v, B_wq, B_wo)
    return f

_impl = make(KP=5, S2=32)


@jax.jit
def pallas_concat_heads__mha_block_cached__mha_block_cached__near_ridge_kernel(
    A_x, A_k_cache, A_v_cache, A_wq, A_wo, B_x, B_k_cache, B_v_cache, B_wq, B_wo
):
    return _impl(A_x, A_k_cache, A_v_cache, A_wq, A_wo, B_x, B_k_cache, B_v_cache, B_wq, B_wo)
```

```python
import jax
import jax.numpy as jnp
from jax import lax
import jax.experimental.pallas as pl
import jax.experimental.pallas.tpu as pltpu

H, DH = 32, 128
SQ, DM, SK = 192, 512, 512
NBATCH = 16
NB = 4
HG = 4
NG = H // HG
LOG_NG = NG.bit_length() - 1
NBB = NBATCH // NB
NSTEPS = NBB * NG
W = HG * DH
NS = 4
KP = 6
HB = NB * SQ // 2

F32 = jnp.float32
BF16 = jnp.bfloat16
NN = (((1,), (0,)), ((), ()))
NT = (((1,), (1,)), ((), ()))
QSCALE = DH ** -0.5 * 1.4426950408889634

ORDER_FULL = (("C", 0), ("B", 1), ("A", 2), ("D", -1))
ORDER_PRE = (("A", 3), ("D", -1), ("B", 1), ("C", 0))
UNITS = [(br, i, j) for i in range(NB) for j in range(HG) for br in range(2)]


def _kernel(xa, ka, va, wqa, woa, xb, kb, vb, wqb, wob, o_ref,
            xbuf, kvbuf, wqbuf, wobuf, qbuf, acc, obuf,
            xhsem, x0sem, xsem, kvsem, wq0sem, wqsem, wosem, osem):
    X, K, V, WQ, WO = (xa, xb), (ka, kb), (va, vb), (wqa, wqb), (woa, wob)

    def wait(ref, sem):
        pltpu.make_async_copy(ref, ref, sem).wait()

    def start_x(g, br, sem):
        pltpu.make_async_copy(X[br].at[pl.ds(g * (NB * SQ), NB * SQ), :],
                              xbuf.at[g & 1, br], sem).start()

    def start_wq(h, br, sem):
        pltpu.make_async_copy(WQ[br].at[:, pl.ds(h * W, W)], wqbuf.at[h, br], sem).start()

    def start_wo(h):
        for br in range(2):
            pltpu.make_async_copy(WO[br].at[pl.ds(h * W, W), :], wobuf.at[h, br],
                                  wosem.at[h & (NS - 1)]).start()

    def start_kv(step):
        sl = step & (NS - 1)
        h0 = (step & (NG - 1)) * HG
        b0 = (step >> LOG_NG) * NB
        for br in range(2):
            for n, src in enumerate((K[br], V[br])):
                pltpu.make_async_copy(src.at[pl.ds(b0, NB), pl.ds(h0, HG)],
                                      kvbuf.at[sl, 2 * br + n], kvsem.at[sl]).start()

    def issue(t, carry):
        @pl.when(t < 2)
        def _():
            rows = pl.ds(pl.multiple_of(t * HB, HB), HB)
            pltpu.make_async_copy(xa.at[rows, :], xbuf.at[0, 0, rows, :], xhsem.at[t]).start()

        @pl.when(t == 0)
        def _():
            start_wq(0, 0, wq0sem.at[0, 0])

        @pl.when(t == 2)
        def _():
            start_x(0, 1, x0sem)
            start_wq(0, 1, wq0sem.at[0, 1])

        @pl.when(jnp.logical_and(t >= 3, t <= KP + 1))
        def _():
            for br in range(2):
                start_wq(t - 2, br, wq0sem.at[t - 2, br])

        @pl.when(t > KP + 1)
        def _():
            start_kv(t - (KP + 2))
            start_wo(t - (KP + 2))

        return carry

    lax.fori_loop(0, KP + 2 + NS, issue, 0)

    def qproj(h, br, rows):
        r = lax.dot_general(xbuf[0, br, rows, :], wqbuf[h, br], NN, preferred_element_type=F32)
        qbuf[h, br, rows, :] = (r * QSCALE).astype(BF16)

    def q_first(c, carry):
        @pl.when(c == 0)
        def _():
            wait(wqbuf.at[0, 0], wq0sem.at[0, 0])
        wait(xbuf.at[0, 0, pl.ds(0, HB), :], xhsem.at[c])
        qproj(0, 0, pl.ds(pl.multiple_of(c * HB, HB), HB))
        return carry

    def q_rest(h, carry):
        for br in range(2):
            wait(wqbuf.at[h, br], wq0sem.at[h, br])
        for br in range(2):
            qproj(h, br, slice(None))
        return carry

    lax.fori_loop(0, 2, q_first, 0)
    wait(xbuf.at[0, 1], x0sem)
    wait(wqbuf.at[0, 1], wq0sem.at[0, 1])
    qproj(0, 1, slice(None))
    lax.fori_loop(1, KP, q_rest, 0)

    def step_body(step, q_precomputed):
        bb = step >> LOG_NG
        hg = step & (NG - 1)
        slot = step & (NS - 1)
        gp = bb & 1
        group_start = hg == 0

        if q_precomputed:
            wait(wobuf.at[hg], wosem.at[slot])
        else:
            @pl.when(step < NG)
            def _():
                wait(wobuf.at[hg], wosem.at[slot])
                wait(wqbuf.at[hg], wqsem.at[slot])

            @pl.when(group_start)
            def _():
                wait(xbuf.at[gp], xsem)

            @pl.when(jnp.logical_and(group_start, bb >= 2))
            def _():
                wait(obuf.at[gp], osem.at[gp])
        wait(kvbuf.at[slot], kvsem.at[slot])

        q, p, l, o, seen = {}, {}, {}, {}, {}

        def stage_a(u):
            br, i, j = UNITS[u]
            rows, cols = slice(i * SQ, (i + 1) * SQ), slice(j * DH, (j + 1) * DH)
            if q_precomputed:
                q[u] = qbuf[hg, br, rows, cols]
            else:
                r = lax.dot_general(xbuf[gp, br, rows, :], wqbuf[hg, br, :, cols], NN,
                                    preferred_element_type=F32)
                q[u] = (r * QSCALE).astype(BF16)

        def stage_b(u):
            br, i, j = UNITS[u]
            s = lax.dot_general(q[u], kvbuf[slot, 2 * br, i, j], NT, preferred_element_type=F32)
            e = jnp.exp2(s - jnp.max(s, axis=-1, keepdims=True))
            l[u] = jnp.sum(e, axis=-1, keepdims=True)
            p[u] = e.astype(BF16)

        def stage_c(u):
            br, i, j = UNITS[u]
            r = lax.dot_general(p[u], kvbuf[slot, 2 * br + 1, i, j], NN,
                                preferred_element_type=F32)
            inv = pl.reciprocal(l[u], approx=True)
            inv = inv * (2.0 - l[u] * inv)
            o[u] = (r * inv).astype(BF16)

        def stage_d(u):
            br, i, j = UNITS[u]
            cols = slice(br * DM, (br + 1) * DM)
            r = lax.dot_general(o[u], wobuf[hg, br, j * DH:(j + 1) * DH, :], NN,
                                preferred_element_type=F32)
            prev = acc[i, :, cols]
            n = seen.get((br, i), 0)
            seen[(br, i)] = n + 1
            if n == 0:
                prev = jnp.where(group_start, 0.0, prev)
            new = prev + r
            acc[i, :, cols] = new
            if n == HG - 1 and not q_precomputed:
                obuf[gp, i, :, cols] = new.astype(BF16)

                @pl.when(hg == NG - 1)
                def _():
                    pltpu.make_async_copy(obuf.at[gp, i, :, cols],
                                          o_ref.at[bb * NB + i, :, cols], osem.at[gp]).start()

        stages = {"A": stage_a, "B": stage_b, "C": stage_c, "D": stage_d}
        order = ORDER_PRE if q_precomputed else ORDER_FULL
        offs = [off for _, off in order]
        for t in range(-max(offs), len(UNITS) - min(offs)):
            for name, off in order:
                if 0 <= t + off < len(UNITS):
                    stages[name](t + off)

        nxt = step + NS

        @pl.when(nxt < NSTEPS)
        def _():
            start_kv(nxt)

        @pl.when(nxt < NG)
        def _():
            start_wo(nxt)

        @pl.when(jnp.logical_and(nxt >= KP, nxt < NG))
        def _():
            for br in range(2):
                start_wq(nxt, br, wqsem.at[slot])

        @pl.when(jnp.logical_and((nxt & (NG - 1)) == 0, nxt < NSTEPS))
        def _():
            for br in range(2):
                start_x(nxt >> LOG_NG, br, xsem)

    def pre_step(step, carry):
        step_body(step, True)
        return carry

    def full_step(step, carry):
        step_body(step, False)
        return carry

    lax.fori_loop(0, KP, pre_step, 0)
    lax.fori_loop(KP, NSTEPS, full_step, 0)
    wait(obuf.at[0], osem.at[0])
    wait(obuf.at[1], osem.at[1])


@jax.jit
def pallas_concat_heads__mha_block_cached__mha_block_cached__near_ridge_kernel(
    A_x: jax.Array,
    A_k_cache: jax.Array,
    A_v_cache: jax.Array,
    A_wq: jax.Array,
    A_wo: jax.Array,
    B_x: jax.Array,
    B_k_cache: jax.Array,
    B_v_cache: jax.Array,
    B_wq: jax.Array,
    B_wo: jax.Array,
):
    assert A_x.shape == (NBATCH, SQ, DM) and A_k_cache.shape == (NBATCH, H, SK, DH)
    assert NS <= KP < NG
    hbm = pl.BlockSpec(memory_space=pl.ANY)
    dma = pltpu.SemaphoreType.DMA
    return pl.pallas_call(
        _kernel,
        in_specs=[hbm] * 10,
        out_specs=hbm,
        out_shape=jax.ShapeDtypeStruct((NBATCH, SQ, 2 * DM), BF16),
        scratch_shapes=[
            pltpu.VMEM((2, 2, NB * SQ, DM), BF16),
            pltpu.VMEM((NS, 4, NB, HG, SK, DH), BF16),
            pltpu.VMEM((NG, 2, DM, W), BF16),
            pltpu.VMEM((NG, 2, W, DM), BF16),
            pltpu.VMEM((KP, 2, NB * SQ, W), BF16),
            pltpu.VMEM((NB, SQ, 2 * DM), F32),
            pltpu.VMEM((2, NB, SQ, 2 * DM), BF16),
            dma((2,)),
            dma(()),
            dma(()),
            dma((NS,)),
            dma((KP, 2)),
            dma((NS,)),
            dma((NS,)),
            dma((2,)),
        ],
        compiler_params=pltpu.CompilerParams(
            vmem_limit_bytes=110 * 1024 * 1024,
            disable_bounds_checks=True,
            disable_semaphore_checks=True,
        ),
    )(A_x.reshape(NBATCH * SQ, DM), A_k_cache, A_v_cache, A_wq, A_wo,
      B_x.reshape(NBATCH * SQ, DM), B_k_cache, B_v_cache, B_wq, B_wo)
```

```python
import jax
import jax.numpy as jnp
from jax import lax
import jax.experimental.pallas as pl
import jax.experimental.pallas.tpu as pltpu

H, DH = 32, 128
SQ, DM, SK = 192, 512, 512
NBATCH = 16
NB = 4
HG = 4
NG = H // HG
LOG_NG = NG.bit_length() - 1
NBB = NBATCH // NB
NSTEPS = NBB * NG
W = HG * DH
NS = 4
KP = 6
HB = NB * SQ // 2

F32 = jnp.float32
BF16 = jnp.bfloat16
NN = (((1,), (0,)), ((), ()))
NT = (((1,), (1,)), ((), ()))
QSCALE = DH ** -0.5 * 1.4426950408889634

ORDER_FULL = (("C", 0), ("B", 1), ("A", 2), ("D", -1))
ORDER_PRE = (("A", 3), ("D", -1), ("B", 1), ("C", 0))
UNITS = [(br, i, j) for i in range(NB) for j in range(HG) for br in range(2)]


def _kernel(xa, ka, va, wqa, woa, xb, kb, vb, wqb, wob, o_ref,
            xbuf, kvbuf, wqbuf, wobuf, qbuf, acc, obuf,
            xhsem, x0sem, xsem, kvsem, wq0sem, wqsem, wosem, osem):
    X, K, V, WQ, WO = (xa, xb), (ka, kb), (va, vb), (wqa, wqb), (woa, wob)

    def wait(ref, sem):
        pltpu.make_async_copy(ref, ref, sem).wait()

    def wait_out(g):
        pltpu.make_async_copy(obuf.at[g & 1], o_ref.at[pl.ds(g * NB, NB)], osem.at[g & 1]).wait()

    def start_x(g, br, sem):
        pltpu.make_async_copy(X[br].at[pl.ds(g * (NB * SQ), NB * SQ), :],
                              xbuf.at[g & 1, br], sem).start()

    def start_wq(h, br, sem):
        pltpu.make_async_copy(WQ[br].at[:, pl.ds(h * W, W)], wqbuf.at[h, br], sem).start()

    def start_wo(h):
        for br in range(2):
            pltpu.make_async_copy(WO[br].at[pl.ds(h * W, W), :], wobuf.at[h, br],
                                  wosem.at[h & (NS - 1)]).start()

    def start_kv(step):
        sl = step & (NS - 1)
        h0 = (step & (NG - 1)) * HG
        b0 = (step >> LOG_NG) * NB
        for br in range(2):
            for n, src in enumerate((K[br], V[br])):
                pltpu.make_async_copy(src.at[pl.ds(b0, NB), pl.ds(h0, HG)],
                                      kvbuf.at[sl, 2 * br + n], kvsem.at[sl]).start()

    def issue(t, carry):
        @pl.when(t < 2)
        def _():
            rows = pl.ds(pl.multiple_of(t * HB, HB), HB)
            pltpu.make_async_copy(xa.at[rows, :], xbuf.at[0, 0, rows, :], xhsem.at[t]).start()

        @pl.when(t == 0)
        def _():
            start_wq(0, 0, wq0sem.at[0, 0])

        @pl.when(t == 2)
        def _():
            start_x(0, 1, x0sem)
            start_wq(0, 1, wq0sem.at[0, 1])

        @pl.when(jnp.logical_and(t >= 3, t <= KP + 1))
        def _():
            for br in range(2):
                start_wq(t - 2, br, wq0sem.at[t - 2, br])

        @pl.when(t > KP + 1)
        def _():
            start_kv(t - (KP + 2))
            start_wo(t - (KP + 2))

        return carry

    lax.fori_loop(0, KP + 2 + NS, issue, 0)

    def qproj(h, br, rows):
        r = lax.dot_general(xbuf[0, br, rows, :], wqbuf[h, br], NN, preferred_element_type=F32)
        qbuf[h, br, rows, :] = (r * QSCALE).astype(BF16)

    def q_first(c, carry):
        @pl.when(c == 0)
        def _():
            wait(wqbuf.at[0, 0], wq0sem.at[0, 0])
        rows = pl.ds(pl.multiple_of(c * HB, HB), HB)
        wait(xbuf.at[0, 0, rows, :], xhsem.at[c])
        qproj(0, 0, rows)
        return carry

    def q_rest(h, carry):
        for br in range(2):
            wait(wqbuf.at[h, br], wq0sem.at[h, br])
        for br in range(2):
            qproj(h, br, slice(None))
        return carry

    lax.fori_loop(0, 2, q_first, 0)
    wait(xbuf.at[0, 1], x0sem)
    wait(wqbuf.at[0, 1], wq0sem.at[0, 1])
    qproj(0, 1, slice(None))
    lax.fori_loop(1, KP, q_rest, 0)

    def step_body(step, q_precomputed):
        bb = step >> LOG_NG
        hg = step & (NG - 1)
        slot = step & (NS - 1)
        gp = bb & 1
        group_start = hg == 0

        if q_precomputed:
            wait(wobuf.at[hg], wosem.at[slot])
        else:
            @pl.when(step < NG)
            def _():
                wait(wobuf.at[hg], wosem.at[slot])
                wait(wqbuf.at[hg], wqsem.at[slot])

            @pl.when(group_start)
            def _():
                wait(xbuf.at[gp], xsem)

            @pl.when(jnp.logical_and(group_start, bb >= 2))
            def _():
                wait_out(bb - 2)
        wait(kvbuf.at[slot], kvsem.at[slot])

        q, p, l, o, seen = {}, {}, {}, {}, {}

        def stage_a(u):
            br, i, j = UNITS[u]
            rows, cols = slice(i * SQ, (i + 1) * SQ), slice(j * DH, (j + 1) * DH)
            if q_precomputed:
                q[u] = qbuf[hg, br, rows, cols]
            else:
                r = lax.dot_general(xbuf[gp, br, rows, :], wqbuf[hg, br, :, cols], NN,
                                    preferred_element_type=F32)
                q[u] = (r * QSCALE).astype(BF16)

        def stage_b(u):
            br, i, j = UNITS[u]
            s = lax.dot_general(q[u], kvbuf[slot, 2 * br, i, j], NT, preferred_element_type=F32)
            e = jnp.exp2(s - jnp.max(s, axis=-1, keepdims=True))
            l[u] = jnp.sum(e, axis=-1, keepdims=True)
            p[u] = e.astype(BF16)

        def stage_c(u):
            br, i, j = UNITS[u]
            r = lax.dot_general(p[u], kvbuf[slot, 2 * br + 1, i, j], NN,
                                preferred_element_type=F32)
            inv = pl.reciprocal(l[u], approx=True)
            inv = inv * (2.0 - l[u] * inv)
            o[u] = (r * inv).astype(BF16)

        def stage_d(u):
            br, i, j = UNITS[u]
            cols = slice(br * DM, (br + 1) * DM)
            r = lax.dot_general(o[u], wobuf[hg, br, j * DH:(j + 1) * DH, :], NN,
                                preferred_element_type=F32)
            prev = acc[i, :, cols]
            n = seen.get((br, i), 0)
            seen[(br, i)] = n + 1
            if n == 0:
                prev = jnp.where(group_start, 0.0, prev)
            new = prev + r
            acc[i, :, cols] = new
            if n == HG - 1 and not q_precomputed:
                obuf[gp, i, :, cols] = new.astype(BF16)

                @pl.when(hg == NG - 1)
                def _():
                    pltpu.make_async_copy(obuf.at[gp, i, :, cols],
                                          o_ref.at[bb * NB + i, :, cols], osem.at[gp]).start()

        stages = {"A": stage_a, "B": stage_b, "C": stage_c, "D": stage_d}
        order = ORDER_PRE if q_precomputed else ORDER_FULL
        offs = [off for _, off in order]
        for t in range(-max(offs), len(UNITS) - min(offs)):
            for name, off in order:
                if 0 <= t + off < len(UNITS):
                    stages[name](t + off)

        nxt = step + NS

        @pl.when(nxt < NSTEPS)
        def _():
            start_kv(nxt)

        @pl.when(nxt < NG)
        def _():
            start_wo(nxt)

        @pl.when(jnp.logical_and(nxt >= KP, nxt < NG))
        def _():
            for br in range(2):
                start_wq(nxt, br, wqsem.at[slot])

        @pl.when(jnp.logical_and((nxt & (NG - 1)) == 0, nxt < NSTEPS))
        def _():
            for br in range(2):
                start_x(nxt >> LOG_NG, br, xsem)

    def pre_step(step, carry):
        step_body(step, True)
        return carry

    def full_step(step, carry):
        step_body(step, False)
        return carry

    lax.fori_loop(0, KP, pre_step, 0)
    lax.fori_loop(KP, NSTEPS, full_step, 0)
    wait_out(NBB - 2)
    wait_out(NBB - 1)


@jax.jit
def pallas_concat_heads__mha_block_cached__mha_block_cached__near_ridge_kernel(
    A_x: jax.Array,
    A_k_cache: jax.Array,
    A_v_cache: jax.Array,
    A_wq: jax.Array,
    A_wo: jax.Array,
    B_x: jax.Array,
    B_k_cache: jax.Array,
    B_v_cache: jax.Array,
    B_wq: jax.Array,
    B_wo: jax.Array,
):
    assert A_x.shape == (NBATCH, SQ, DM) and A_k_cache.shape == (NBATCH, H, SK, DH)
    assert NS <= KP < NG
    hbm = pl.BlockSpec(memory_space=pl.ANY)
    dma = pltpu.SemaphoreType.DMA
    return pl.pallas_call(
        _kernel,
        in_specs=[hbm] * 10,
        out_specs=hbm,
        out_shape=jax.ShapeDtypeStruct((NBATCH, SQ, 2 * DM), BF16),
        scratch_shapes=[
            pltpu.VMEM((2, 2, NB * SQ, DM), BF16),
            pltpu.VMEM((NS, 4, NB, HG, SK, DH), BF16),
            pltpu.VMEM((NG, 2, DM, W), BF16),
            pltpu.VMEM((NG, 2, W, DM), BF16),
            pltpu.VMEM((KP, 2, NB * SQ, W), BF16),
            pltpu.VMEM((NB, SQ, 2 * DM), F32),
            pltpu.VMEM((2, NB, SQ, 2 * DM), BF16),
            dma((2,)),
            dma(()),
            dma(()),
            dma((NS,)),
            dma((KP, 2)),
            dma((NS,)),
            dma((NS,)),
            dma((2,)),
        ],
        compiler_params=pltpu.CompilerParams(
            vmem_limit_bytes=110 * 1024 * 1024,
            disable_bounds_checks=True,
            disable_semaphore_checks=True,
        ),
    )(A_x.reshape(NBATCH * SQ, DM), A_k_cache, A_v_cache, A_wq, A_wo,
      B_x.reshape(NBATCH * SQ, DM), B_k_cache, B_v_cache, B_wq, B_wo)
```

```python
import jax
import jax.numpy as jnp
from jax import lax
import jax.experimental.pallas as pl
import jax.experimental.pallas.tpu as pltpu

H, DH = 32, 128
SQ, DM, SK = 192, 512, 512
NBATCH = 16
NB = 4
HG = 4
NG = H // HG
LOG_NG = NG.bit_length() - 1
NBB = NBATCH // NB
NSTEPS = NBB * NG
W = HG * DH
NS = 4
KP = 6
HB = NB * SQ // 2

F32 = jnp.float32
BF16 = jnp.bfloat16
NN = (((1,), (0,)), ((), ()))
NT = (((1,), (1,)), ((), ()))
QSCALE = DH ** -0.5 * 1.4426950408889634

ORDER_FULL = (("C", 0), ("B", 1), ("A", 2), ("D", -1))
ORDER_PRE = (("A", 3), ("D", -1), ("B", 1), ("C", 0))
UNITS = [(br, i, j) for i in range(NB) for j in range(HG) for br in range(2)]


def _kernel(xa, ka, va, wqa, woa, xb, kb, vb, wqb, wob, o_ref,
            xbuf, kvbuf, wbuf, qbuf, acc, obuf,
            xhsem, x0sem, xsem, kvsem, wq0sem, wsem, osem):
    X, K, V, WQ, WO = (xa, xb), (ka, kb), (va, vb), (wqa, wqb), (woa, wob)

    def wait(ref, sem):
        pltpu.make_async_copy(ref, ref, sem).wait()

    def start_x(g, br, sem):
        pltpu.make_async_copy(X[br].at[pl.ds(g * (NB * SQ), NB * SQ), :],
                              xbuf.at[g & 1, br], sem).start()

    def start_wq(h, br, sem):
        pltpu.make_async_copy(WQ[br].at[:, pl.ds(h * W, W)], wbuf.at[h, 0, br], sem).start()

    def start_wo(h):
        for br in range(2):
            pltpu.make_async_copy(WO[br].at[pl.ds(h * W, W), :], wbuf.at[h, 1, br],
                                  wsem.at[h & (NS - 1)]).start()

    def start_kv(step):
        sl = step & (NS - 1)
        h0 = (step & (NG - 1)) * HG
        b0 = (step >> LOG_NG) * NB
        for br in range(2):
            for n, src in enumerate((K[br], V[br])):
                pltpu.make_async_copy(src.at[pl.ds(b0, NB), pl.ds(h0, HG)],
                                      kvbuf.at[sl, 2 * br + n], kvsem.at[sl]).start()

    def issue(t, carry):
        @pl.when(t < 2)
        def _():
            rows = pl.ds(pl.multiple_of(t * HB, HB), HB)
            pltpu.make_async_copy(xa.at[rows, :], xbuf.at[0, 0, rows, :], xhsem.at[t]).start()

        @pl.when(t == 0)
        def _():
            start_wq(0, 0, wq0sem.at[0, 0])

        @pl.when(t == 2)
        def _():
            start_x(0, 1, x0sem)
            start_wq(0, 1, wq0sem.at[0, 1])

        @pl.when(jnp.logical_and(t >= 3, t <= KP + 1))
        def _():
            for br in range(2):
                start_wq(t - 2, br, wq0sem.at[t - 2, br])

        @pl.when(t > KP + 1)
        def _():
            start_kv(t - (KP + 2))
            start_wo(t - (KP + 2))

        return carry

    lax.fori_loop(0, KP + 2 + NS, issue, 0)

    def qproj(h, br, rows):
        r = lax.dot_general(xbuf[0, br, rows, :], wbuf[h, 0, br], NN, preferred_element_type=F32)
        qbuf[h, br, rows, :] = (r * QSCALE).astype(BF16)

    def q_first(c, carry):
        @pl.when(c == 0)
        def _():
            wait(wbuf.at[0, 0, 0], wq0sem.at[0, 0])
        rows = pl.ds(pl.multiple_of(c * HB, HB), HB)
        wait(xbuf.at[0, 0, rows, :], xhsem.at[c])
        qproj(0, 0, rows)
        return carry

    def q_rest(h, carry):
        for br in range(2):
            wait(wbuf.at[h, 0, br], wq0sem.at[h, br])
        for br in range(2):
            qproj(h, br, slice(None))
        return carry

    lax.fori_loop(0, 2, q_first, 0)
    wait(xbuf.at[0, 1], x0sem)
    wait(wbuf.at[0, 0, 1], wq0sem.at[0, 1])
    qproj(0, 1, slice(None))
    lax.fori_loop(1, KP, q_rest, 0)

    def step_body(step, q_precomputed):
        bb = step >> LOG_NG
        hg = step & (NG - 1)
        slot = step & (NS - 1)
        gp = bb & 1
        group_start = hg == 0

        if q_precomputed:
            wait(wbuf.at[hg, 1], wsem.at[slot])
        else:
            @pl.when(step < NG)
            def _():
                wait(wbuf.at[hg], wsem.at[slot])

            @pl.when(group_start)
            def _():
                wait(xbuf.at[gp], xsem)
        wait(kvbuf.at[slot], kvsem.at[slot])

        q, p, l, o, seen = {}, {}, {}, {}, {}

        def stage_a(u):
            br, i, j = UNITS[u]
            rows, cols = slice(i * SQ, (i + 1) * SQ), slice(j * DH, (j + 1) * DH)
            if q_precomputed:
                q[u] = qbuf[hg, br, rows, cols]
            else:
                r = lax.dot_general(xbuf[gp, br, rows, :], wbuf[hg, 0, br, :, cols], NN,
                                    preferred_element_type=F32)
                q[u] = (r * QSCALE).astype(BF16)

        def stage_b(u):
            br, i, j = UNITS[u]
            s = lax.dot_general(q[u], kvbuf[slot, 2 * br, i, j], NT, preferred_element_type=F32)
            e = jnp.exp2(s - jnp.max(s, axis=-1, keepdims=True))
            l[u] = jnp.sum(e, axis=-1, keepdims=True)
            p[u] = e.astype(BF16)

        def stage_c(u):
            br, i, j = UNITS[u]
            r = lax.dot_general(p[u], kvbuf[slot, 2 * br + 1, i, j], NN,
                                preferred_element_type=F32)
            inv = pl.reciprocal(l[u], approx=True)
            inv = inv * (2.0 - l[u] * inv)
            o[u] = (r * inv).astype(BF16)

        def stage_d(u):
            br, i, j = UNITS[u]
            cols = slice(br * DM, (br + 1) * DM)
            r = lax.dot_general(o[u], wbuf[hg, 1, br, j * DH:(j + 1) * DH, :], NN,
                                preferred_element_type=F32)
            prev = acc[i, :, cols]
            n = seen.get((br, i), 0)
            seen[(br, i)] = n + 1
            if n == 0:
                prev = jnp.where(group_start, 0.0, prev)
            new = prev + r
            acc[i, :, cols] = new
            if n == HG - 1 and not q_precomputed:
                b = bb * NB + i
                obuf[b, :, cols] = new.astype(BF16)

                @pl.when(hg == NG - 1)
                def _():
                    pltpu.make_async_copy(obuf.at[b, :, cols], o_ref.at[b, :, cols], osem).start()

        stages = {"A": stage_a, "B": stage_b, "C": stage_c, "D": stage_d}
        order = ORDER_PRE if q_precomputed else ORDER_FULL
        offs = [off for _, off in order]
        for t in range(-max(offs), len(UNITS) - min(offs)):
            for name, off in order:
                if 0 <= t + off < len(UNITS):
                    stages[name](t + off)

        nxt = step + NS

        @pl.when(nxt < NSTEPS)
        def _():
            start_kv(nxt)

        @pl.when(nxt < NG)
        def _():
            start_wo(nxt)

        @pl.when(jnp.logical_and(nxt >= KP, nxt < NG))
        def _():
            for br in range(2):
                start_wq(nxt, br, wsem.at[slot])

        @pl.when(jnp.logical_and((nxt & (NG - 1)) == 0, nxt < NSTEPS))
        def _():
            for br in range(2):
                start_x(nxt >> LOG_NG, br, xsem)

    def pre_step(step, carry):
        step_body(step, True)
        return carry

    def full_step(step, carry):
        step_body(step, False)
        return carry

    lax.fori_loop(0, KP, pre_step, 0)
    lax.fori_loop(KP, NSTEPS, full_step, 0)
    pltpu.make_async_copy(obuf, o_ref, osem).wait()


@jax.jit
def pallas_concat_heads__mha_block_cached__mha_block_cached__near_ridge_kernel(
    A_x: jax.Array,
    A_k_cache: jax.Array,
    A_v_cache: jax.Array,
    A_wq: jax.Array,
    A_wo: jax.Array,
    B_x: jax.Array,
    B_k_cache: jax.Array,
    B_v_cache: jax.Array,
    B_wq: jax.Array,
    B_wo: jax.Array,
):
    assert A_x.shape == (NBATCH, SQ, DM) and A_k_cache.shape == (NBATCH, H, SK, DH)
    assert NS <= KP < NG and W == DM
    hbm = pl.BlockSpec(memory_space=pl.ANY)
    dma = pltpu.SemaphoreType.DMA
    return pl.pallas_call(
        _kernel,
        in_specs=[hbm] * 10,
        out_specs=hbm,
        out_shape=jax.ShapeDtypeStruct((NBATCH, SQ, 2 * DM), BF16),
        scratch_shapes=[
            pltpu.VMEM((2, 2, NB * SQ, DM), BF16),
            pltpu.VMEM((NS, 4, NB, HG, SK, DH), BF16),
            pltpu.VMEM((NG, 2, 2, DM, W), BF16),
            pltpu.VMEM((KP, 2, NB * SQ, W), BF16),
            pltpu.VMEM((NB, SQ, 2 * DM), F32),
            pltpu.VMEM((NBATCH, SQ, 2 * DM), BF16),
            dma((2,)),
            dma(()),
            dma(()),
            dma((NS,)),
            dma((KP, 2)),
            dma((NS,)),
            dma(()),
        ],
        compiler_params=pltpu.CompilerParams(
            vmem_limit_bytes=110 * 1024 * 1024,
            disable_bounds_checks=True,
            disable_semaphore_checks=True,
        ),
    )(A_x.reshape(NBATCH * SQ, DM), A_k_cache, A_v_cache, A_wq, A_wo,
      B_x.reshape(NBATCH * SQ, DM), B_k_cache, B_v_cache, B_wq, B_wo)
```
